```python
import jax
import jax.numpy as jnp

def _softmax(x, axis=-1):
    return jax.nn.softmax(x, axis=axis)

def _gelu(x):
    return jax.nn.gelu(x, approximate=True)

def _silu(x):
    return jax.nn.silu(x)

def _sigmoid(x):
    return jax.nn.sigmoid(x)

def _layernorm(x, axis=-1, eps=1e-05):
    m = jnp.mean(x, axis=axis, keepdims=True)
    v = jnp.var(x, axis=axis, keepdims=True)
    return (x - m) / jnp.sqrt(v + eps)

def _scatter_add(tgt, idx, src, axis=0):
    return tgt.at[idx].add(src)

def _segment_sum(src, seg, n):
    return jax.ops.segment_sum(src, seg, n)

class _Rng:

    def __init__(self, key):
        self._k = key

    def _next(self):
        self._k, sub = jax.random.split(self._k)
        return sub

    def normal(self, shape):
        return jax.random.normal(self._next(), shape, dtype=jnp.bfloat16)

    def randint(self, lo, hi, shape):
        return jax.random.randint(self._next(), shape, lo, hi, dtype=jnp.int32)

    def uniform(self, shape, lo=0.0, hi=1.0):
        return jax.random.uniform(self._next(), shape, jnp.bfloat16, lo, hi)

    def permutation(self, n):
        return jax.random.permutation(self._next(), n)
kernel_name = 'adaLN_cond__grouped_kv_mqa__mixer_token_mlp__prompt'

def _fwd_setup_inputs():
    _rng = _Rng(jax.random.key(int.from_bytes(__import__("os").urandom(4), "little")))
    _w = lambda a: (lambda t: t.astype(jnp.bfloat16) if jnp.issubdtype(t.dtype, jnp.floating) else t)(jnp.asarray(a))

    def _A_setup():
        B, S, D, H = (1, 2048, 512, 32)
        Dh = D // H
        return {'x': _w((lambda *s: _rng.normal(s) * 0.05)(B, S, D)), 'wq': _w((lambda *s: _rng.normal(s) * 0.05)(D, H * Dh)), 'wk': _w((lambda *s: _rng.normal(s) * 0.05)(D, Dh)), 'wv': _w((lambda *s: _rng.normal(s) * 0.05)(D, Dh)), 'wo': _w((lambda *s: _rng.normal(s) * 0.05)(H * Dh, D))}
    _A_in = _A_setup()

    def _B_setup():
        B, S, D, F = (1, 2048, 512, 1376)
        return {'x': _w((lambda *s: _rng.normal(s) * 0.05)(B, S, D)), 'w1': _w((lambda *s: _rng.normal(s) * 0.05)(S, F) * S ** (-0.5)), 'b1': _w((lambda *s: _rng.normal(s) * 0.05)(F) * 0.02), 'w2': _w((lambda *s: _rng.normal(s) * 0.05)(F, S) * F ** (-0.5)), 'b2': _w((lambda *s: _rng.normal(s) * 0.05)(S) * 0.02)}
    _B_in = _B_setup()
    return {'A_x': _A_in['x'], 'A_wq': _A_in['wq'], 'A_wk': _A_in['wk'], 'A_wv': _A_in['wv'], 'A_wo': _A_in['wo'], 'B_x': _B_in['x'], 'B_w1': _B_in['w1'], 'B_b1': _B_in['b1'], 'B_w2': _B_in['w2'], 'B_b2': _B_in['b2'], 'c': _w((lambda *s: _rng.normal(s) * 0.05)(1, 512)), 'w_mod': _w((lambda *s: _rng.normal(s) * 0.05)(512, 6 * 512) * 512 ** (-0.5))}

def _fwd_reference(A_x, A_wq, A_wk, A_wv, A_wo, B_x, B_w1, B_b1, B_w2, B_b2, c, w_mod):

    def _A_ref(x, wq, wk, wv, wo):
        B, S, D = x.shape
        H = 32
        Dh = D // H
        q = (lambda x, *d: x.transpose(*d))((x @ wq).reshape(B, S, H, Dh), 0, 2, 1, 3)
        k = x @ wk
        v = x @ wv
        scores = jnp.einsum('bhqd,bkd->bhqk', q, k) * Dh ** (-0.5)
        p = _softmax(scores, axis=-1)
        o = jnp.einsum('bhqk,bkd->bhqd', p, v)
        return (lambda x, *d: x.transpose(*d))(o, 0, 2, 1, 3).reshape(B, S, H * Dh) @ wo

    def _B_ref(x, w1, b1, w2, b2):
        B, S, D = x.shape
        h = _layernorm(x, axis=-1)
        u = jnp.einsum('bsd,sf->bdf', h, w1) + b1
        u = _gelu(u)
        y = jnp.einsum('bdf,fs->bds', u, w2) + b2
        return (lambda x, *d: x.transpose(*d))(y, 0, 2, 1)
    x = A_x
    mod = (_silu(c) @ w_mod).reshape(c.shape[0], 6, 1, -1)
    sa, ca, ga, sb, cb, gb = (mod[:, 0].copy(), mod[:, 1].copy(), mod[:, 2].copy(), mod[:, 3].copy(), mod[:, 4].copy(), mod[:, 5].copy())
    h = _layernorm(x, axis=-1) * (1 + ca) + sa
    x = x + ga * _A_ref(h, A_wq, A_wk, A_wv, A_wo)
    h = _layernorm(x, axis=-1) * (1 + cb) + sb
    x = x + gb * _B_ref(h, B_w1, B_b1, B_w2, B_b2)
    return x

def setup_inputs():
    _inp = _fwd_setup_inputs()
    _gk = jax.random.fold_in(jax.random.key(int.from_bytes(__import__("os").urandom(4), "little")), 2 ** 31 - 1)
    _shapes = [[1, 2048, 512]]
    _dtypes = ['bfloat16']
    _gks = jax.random.split(_gk, len(_shapes))
    _gs = [jax.random.normal(k, s, dtype=jnp.dtype(d)) * 0.05 for k, s, d in zip(_gks, _shapes, _dtypes)]
    _inp['grad_out'] = _gs[0]
    return _inp

def reference(A_x, A_wq, A_wk, A_wv, A_wo, B_w1, B_b1, B_w2, B_b2, c, w_mod, B_x, grad_out):
    _const = dict(B_x=B_x)

    def _f(*_d):
        return _fwd_reference(**{'A_x': _d[0], 'A_wq': _d[1], 'A_wk': _d[2], 'A_wv': _d[3], 'A_wo': _d[4], 'B_w1': _d[5], 'B_b1': _d[6], 'B_w2': _d[7], 'B_b2': _d[8], 'c': _d[9], 'w_mod': _d[10], **_const})
    _out, _vjp = jax.vjp(_f, A_x, A_wq, A_wk, A_wv, A_wo, B_w1, B_b1, B_w2, B_b2, c, w_mod)
    _grads = _vjp(grad_out)
    _out0 = jnp.asarray(_out)
    return (_out0, *[jnp.asarray(_g) for _g in _grads])
```

```python
import math

import jax
import jax.numpy as jnp
from jax import lax
import jax.experimental.pallas as pl
import jax.experimental.pallas.tpu as pltpu

f32 = jnp.float32
bf16 = jnp.bfloat16
u32 = jnp.uint32

S, D, H, DH, F = 2048, 512, 32, 16, 1376
EPS = 1e-5
QK_SCALE = DH ** -0.5
LOG2E = math.log2(math.e)
LN2 = math.log(2.0)

BQ = 512
CK = 128
NQ = S // BQ
NC = S // CK
NSTEP = H * NQ
UF = 4
HEAD = (1, 1)
TAIL = (1, 1)
UB = 8
UR = 4
NSLOT = 54
NSAVE = 116
NREC = NSTEP - NSAVE
NHBM = NSAVE - NSLOT
NLEND = 5
LAG = 2
DEP = 7
TB = 256
NTB = S // TB
FB = 256
FT = F // 16
SPLIT = 768
RING = UF * NC // 3
assert NTB == 2 * (NLEND - 1) and NREC <= 3 * NQ and RING > NC + LAG
assert NSAVE <= 3 * NSLOT and NSLOT % 2 == NSAVE % 2 == UB % 2 == 0
assert HEAD[0] == TAIL[-1] == 1 and sum(TAIL) >= 2
assert (NSTEP - sum(HEAD) - sum(TAIL)) % UF == 0


def _mm(a, b):
    return jnp.dot(a, b, preferred_element_type=f32)


def _mm_nt(a, b):
    return lax.dot_general(a, b, (((1,), (1,)), ((), ())), preferred_element_type=f32)


def _mm_rows(a, b, mm=_mm, rows=128):
    return jnp.concatenate([mm(a[i:i + rows], b) for i in range(0, a.shape[0], rows)], axis=0)


def _ds(i, n):
    if isinstance(i, int):
        return pl.ds(i * n, n)
    return pl.ds(pl.multiple_of(i * n, n), n)


def _div(i, n):
    return i // n if isinstance(i, int) else lax.div(i, jnp.int32(n))


def _rem(i, n):
    return i % n if isinstance(i, int) else lax.rem(i, jnp.int32(n))


def _slot(b):
    if isinstance(b, int):
        return b % NSLOT
    return b - jnp.where(b >= NSLOT, NSLOT, 0) - jnp.where(b >= 2 * NSLOT, NSLOT, 0)


def _when(cond, fn):
    if isinstance(cond, bool):
        if cond:
            fn()
    else:
        pl.when(cond)(fn)


def _start(*copies):
    for d in copies:
        d.start()


def _wait(*copies):
    for d in copies:
        d.wait()


def _after(v, z):
    return jnp.maximum(v, jnp.minimum(v, z))


def _accumulate(step, acc, x):
    return jnp.where(step == 0, 0.0, acc) + x


def _col(row):
    return jnp.broadcast_to(row, (128, row.shape[1])).T


def _wide(col, n):
    return jnp.concatenate([col] * (n // 128), axis=1)


def _fold(x):
    acc = x[:, 0:128]
    for i in range(1, x.shape[1] // 128):
        acc = acc + x[:, i * 128:(i + 1) * 128]
    return acc


def _row(partial):
    return jnp.sum(partial.T, axis=0, keepdims=True)


def _mean0(x):
    return jnp.sum(x, axis=0, keepdims=True) * (1.0 / x.shape[0])


def _paced(v, pace, n):
    if pace is None:
        return v
    z, first, step, groups = pace
    return jnp.concatenate(
        [jnp.broadcast_to(_after(v, z[i:i + 1, 0:v.shape[1]]), (n // groups, v.shape[1]))
         for i in range(first, first + step * groups, step)], axis=0)


def _ln(x, pace=None):
    mu = _mean0(x)
    xc = x - _paced(mu, pace, x.shape[0])
    r = lax.rsqrt(_mean0(xc * xc) + EPS)
    return xc * r, mu, r


def _ln_bwd(dy, xhat, r, pace=None):
    a, b = _mean0(dy), _mean0(dy * xhat)
    return r * (dy - _paced(a, pace, dy.shape[0]) - xhat * _paced(b, pace, dy.shape[0]))


def _rows_by_head_dim(xt):
    pad = jnp.concatenate([xt, jnp.zeros((128 - DH, xt.shape[1]), f32)], axis=0)
    return pltpu.bitcast(pad.T.astype(bf16), f32)


def _to16(v):
    return v.reshape(v.shape[0] // 16, 16, v.shape[1]).astype(bf16)


def _from16(v):
    return v.reshape(v.shape[0] * 16, v.shape[2])


def _kernel(x_hbm, wq_hbm, wkT_hbm, wvT_hbm, wo_hbm, w1T_hbm, b1_hbm, w2_hbm, b2_hbm,
            c_hbm, wmod_hbm, go_hbm,
            out_hbm, dx_hbm, dwq_hbm, dwkT_hbm, dwvT_hbm, dwo_hbm, dw1T_hbm, db1_hbm,
            dw2_hbm, db2_hbm, dc_hbm, dwmod_hbm, p_hbm, lent_hbm, q_hbm,
            p_buf, xT, oT, k_buf, kvT, l_buf, rows, mod_buf, dmod_buf, col, c_buf, b1_buf,
            b2_buf, w1s, h_buf, gin, wsq, wkv, p_sem, w_sem, sem):
    cp = pltpu.make_async_copy
    B1, B2, MU, RSTD, MAX = range(5)

    def mod_row(i):
        return mod_buf[:, i * D:(i + 1) * D]

    def step_slices(t):
        return _ds(_div(t, NQ), DH), _ds(_rem(t, NQ), BQ), pl.ds(_div(t, NQ), 1)

    def max_slices(t):
        kept = (t >= NSLOT) & (t < NSLOT + NREC)
        return pl.ds(jnp.where(kept, MAX + _div(t - NSLOT, NQ), 7), 1), _ds(_rem(t, NQ), BQ)

    def p_write(b):
        return cp(p_buf.at[_slot(b)], p_hbm.at[b], p_sem.at[_slot(b)])

    def p_read(b):
        return cp(p_hbm.at[pl.ds(b, 2)], p_buf.at[pl.ds(_slot(b), 2)], p_sem.at[_slot(b)])

    def lend(i, quarter):
        part, slot = _ds(quarter, S // 64), _slot(NHBM + i)
        return cp(p_buf.at[slot, part], lent_hbm.at[i, part], p_sem.at[slot])

    def repay(i):
        slot = _slot(NHBM + i)
        return cp(lent_hbm.at[i], p_buf.at[slot, pl.ds(0, 3 * S // 64)], p_sem.at[slot])

    def tile(slot, i):
        return p_buf.at[slot + _div(i, 4), _ds(_rem(i, 4), D // 16)]

    def x_load(slot, j):
        return cp(x_hbm.at[_ds(j, BQ // 16)], tile(slot, j), sem.at[4 + j])

    def wmod_load(slot, i):
        return cp(wmod_hbm.at[:, :, pl.ds(i * D, D)], tile(slot, i), sem.at[8 + i])

    def w1_load(j, slot):
        return cp(w1T_hbm.at[:, _ds(j, TB)], w1s.at[slot], w_sem.at[1, slot])

    def g_load(j, slot):
        return cp(go_hbm.at[_ds(j, TB)], gin.at[slot], w_sem.at[2, slot])

    def head_rows(buf, c):
        return pltpu.bitcast(buf[pl.ds(c * (CK // 2), CK // 2), 0:DH], bf16)

    def head_cols(i, c):
        return pltpu.bitcast(kvT[i * (DH // 2):(i + 1) * (DH // 2), pl.ds(c * CK, CK)], bf16)

    def modulated(x, tok):
        xhat = (x.astype(f32) - rows[MU:MU + 1, tok]) * rows[RSTD:RSTD + 1, tok]
        n = x.shape[1]
        return xhat, (xhat * _wide(col[1], n) + _wide(col[0], n)).astype(bf16)

    def attention_out(j):
        tok = _ds(j, TB)
        a = _mm(wsq[...], oT[:, tok])
        xT[:, tok] = (xT[:, tok].astype(f32) + _wide(col[2], TB) * a).astype(bf16)

    def ln23(j, za=None, zb=None):
        xh2, _, r2 = _ln(xT[:, _ds(j, TB)].astype(f32), za)
        h3, _, r3 = _ln(xh2 * _wide(col[1], TB) + _wide(col[0], TB), zb)
        h_buf[...] = _to16(h3)
        return xh2, r2, h3, r3

    c_wo = cp(wo_hbm, wsq, sem.at[14])

    def first_half(s_buf, wqT, h1):
        c_c = cp(c_hbm, c_buf, sem.at[0])
        c_k = cp(wkT_hbm, wkv.at[pl.ds(0, DH)], sem.at[1])
        c_v = cp(wvT_hbm, wkv.at[pl.ds(DH, DH)], sem.at[2])
        c_q = cp(wq_hbm, wsq, sem.at[3])
        c_m = [wmod_load(NSLOT - 3, i) for i in range(6)]
        c_b = [cp(b1_hbm, b1_buf, sem.at[15]), cp(b2_hbm, b2_buf, sem.at[16])]
        c_x = [x_load(NSLOT - 1, j) for j in range(NQ)]
        _start(c_c, *c_m[:2], c_x[0], c_k, c_v, c_q, *c_x[1:], *c_m[2:], *c_b, g_load(0, 0),
               w1_load(0, 0))

        def mod_part(i, lanes):
            cv = c_buf[...].astype(f32)
            sc = jnp.broadcast_to(cv * jax.nn.sigmoid(cv), (16, D)).astype(bf16)
            w = _from16(tile(NSLOT - 3, i)[:, :, lanes])
            mod_buf[:, pl.ds(i * D + lanes.start, lanes.size)] = _mm(sc, w)[0:1]

        _wait(c_c, *c_m[:2])
        mod_part(0, pl.ds(0, D))
        mod_part(1, pl.ds(0, D))
        col[0] = _col(mod_row(0))
        col[1] = _col(1.0 + mod_row(1))

        def normalize(j, q=None):
            for i in range(BQ // 128):
                tok = _ds(j * (BQ // 128) + i, 128)
                xt = _from16(tile(NSLOT - 1, j)[_ds(i, 8)]).T
                xT[:, tok] = xt
                xhat, rows[MU:MU + 1, tok], rows[RSTD:RSTD + 1, tok] = _ln(
                    xt.astype(f32), None if q is None else (q, 96 * i, 32, 4))
                h1[:, _ds(i, 128)] = (xhat * col[1] + col[0]).astype(bf16)

        def project(j):
            tok = _ds(j, BQ)
            kv = _mm(wkv[...], h1[...])
            kvT[:, tok] = pltpu.bitcast(kv.astype(bf16), u32)
            k_buf[_ds(j, BQ // 2), :] = _rows_by_head_dim(kv[0:DH])
            q = _mm_rows(wqT[...], h1[...], rows=64)
            oT[:, tok] = (q * (QK_SCALE * LOG2E)).astype(bf16)
            return q

        def project_body(j, _):
            x_load(NSLOT - 1, j + 1).wait()
            normalize(j + 1, project(j))
            return 0

        c_x[0].wait()
        normalize(0)
        _wait(c_k, c_v, c_q)
        wqT[...] = wsq[...].T
        c_wo.start()
        lax.fori_loop(0, NQ - 1, project_body, 0)
        project(NQ - 1)
        c_qo = [cp(oT.at[:, _ds(j, BQ)], q_hbm.at[:, _ds(j, BQ)], sem.at[j]) for j in range(NQ)]
        _start(*c_qo)
        _wait(*c_m[2:])

        def s_rows(phase, c):
            g = (phase % UF) * NC + c
            return pl.ds((g - min(g // RING, 2) * RING) * CK, CK)

        def s_chunk(q, phase, c, mx, hist):
            s = _mm(head_rows(k_buf, c), q)
            s_buf[s_rows(phase, c), :] = s
            for half in (s[:CK // 2], s[CK // 2:]):
                part = jnp.max(half.reshape(CK // 16, 8, BQ), axis=0)
                mx = part if mx is None else jnp.maximum(mx, part)
                hist.append(mx)
            return mx

        def load_q(t):
            r, cq, _ = step_slices(t)
            return oT[r, cq]

        def saved_index(t):
            if isinstance(t, int):
                return t if t < NSLOT else max(t - NREC, NSLOT)
            return jnp.where(t < NSLOT, t, jnp.maximum(t - NREC, NSLOT))

        def release_slots(t0, count):
            for t in [t0 + u for u in range(count)]:
                b = saved_index(t)
                saved = (t < NSLOT) | (t >= NSLOT + NREC)
                _when(saved & (b < NHBM), lambda: p_write(b).start(priority=1))

        def claim_slots(t0, count):
            slots = []
            for t in [t0 + u for u in range(count)]:
                b = saved_index(t)
                _when((t == NSLOT) | (t > NSLOT + NREC), lambda: p_write(b - NSLOT).wait())
                slots.append(_slot(b))
            return slots

        def blocks(t0, phase, slots, m, mx):
            qs, hist = {}, []
            for u, slot in enumerate(slots):
                r, cq, hr = step_slices(t0 + u)
                m8 = jnp.broadcast_to(m, (8, BQ))
                m_next = l = o = None
                for c in range(NC):
                    du, sc = divmod(u * NC + c + NC + LAG, NC)
                    ahead = not (isinstance(t0, int) and t0 + du >= NSTEP)
                    if ahead:
                        if du not in qs:
                            qs[du] = load_q(t0 + du)
                        mx = s_chunk(qs[du], phase + du, sc, None if sc == 0 else mx, hist)
                        if sc == NC - 1:
                            m_next = jnp.max(mx, axis=0, keepdims=True)
                    k = 2 * (u * NC + c) + 1 - DEP
                    mc = _after(m8, hist[k]) if k >= 0 else m8
                    p = jnp.exp2(s_buf[s_rows(phase + u, c), :]
                                 - jnp.concatenate([mc] * (CK // 8), axis=0))
                    lp = p[CK - 8:CK]
                    for i in reversed(range(CK // 8 - 1)):
                        lp = lp + p[i * 8:(i + 1) * 8]
                    l = lp if l is None else l + lp
                    p_buf[slot, pl.ds(c * (CK // 16), CK // 16)] = _to16(p)
                    op = _mm(head_cols(1, c), p.astype(bf16))
                    o = op if o is None else o + op
                    if not ahead:
                        hist += [op[0:8], op[8:16]]
                linv = 1.0 / jnp.sum(l, axis=0, keepdims=True)
                if isinstance(t0, int) and t0 + u == 0:
                    c_qo[0].wait()
                oT[r, cq] = (o * linv).astype(bf16)
                rows[max_slices(t0 + u)] = m
                l_buf[hr, cq] = linv
                m = m_next
            return m, mx

        q0, mx = load_q(0), None
        for c in range(NC):
            mx = s_chunk(q0, 0, c, mx, [])
            mod_part(2 + c // 4, pl.ds((c % 4) * 128, 128))
        m = jnp.max(mx, axis=0, keepdims=True)
        q1, mx = load_q(1), None
        for c in range(LAG):
            mx = s_chunk(q1, 1, c, mx, [])
        t0 = 0
        for i, n in enumerate(HEAD):
            m, mx = blocks(t0, t0, claim_slots(t0, n), m, mx)
            release_slots(t0, n)
            if i == 0:
                _wait(*c_qo[1:], c_wo, *c_b)
            t0 += n
        first, trips = t0, (NSTEP - sum(HEAD) - sum(TAIL)) // UF

        def body(it, carry):
            t = first + it * UF
            carry = blocks(t, first, claim_slots(t, UF), *carry)
            release_slots(t, UF)
            return carry

        m, mx = lax.fori_loop(0, trips, body, (m, mx))
        t0 = first + trips * UF
        for i, n in enumerate(TAIL):
            slots = claim_slots(t0, n)
            if i == 0:
                col[0] = _col(mod_row(3))
                col[1] = _col(1.0 + mod_row(4))
                col[2] = _col(mod_row(2))
                wsq[...] = wsq[...].T
                rows[B1:B1 + 1, 0:F] = b1_buf[...].astype(f32).reshape(1, F)
                rows[B2:B2 + 1, :] = b2_buf[...].astype(f32).reshape(1, S)
            if i == len(TAIL) - 1:
                _start(*[lend(NLEND - 1, quarter) for quarter in range(3)], g_load(1, 1))
                attention_out(0)
                ln23(0)
            m, mx = blocks(t0, t0, slots, m, mx)
            t0 += n

    pl.run_scoped(first_half, pltpu.VMEM(((UF * NC - 2 * RING) * CK, BQ), f32),
            pltpu.VMEM((D, D), bf16), pltpu.VMEM((D, BQ), bf16))

    lent = [(NHBM + i) % NSLOT for i in range(NLEND)]

    def w2_block(slot):
        return p_buf.at[lent[4], pl.ds(0, FT), :, _ds(slot, TB)]

    def w_loads(j, slot):
        return [cp(w2_hbm.at[:, :, _ds(j, TB)], w2_block(slot), w_sem.at[0, slot]),
                w1_load(j, slot)]

    def mlp_hidden(goT, u_acc, w2r, r_sem):
        def w2_rows(i, n, slot):
            return cp(w2_hbm.at[pl.ds(i * (FB // 16), n // 16)],
                      w2r.at[slot, pl.ds(0, n // 16)], r_sem.at[slot])

        g_load(0, 0).wait()
        lend(0, 0).start(priority=1)
        goT[:, 0:TB] = gin[0].T

        def mix_body(j, _):
            slot = lax.rem(j, 2)
            w1_load(j + 1, 1 - slot).start()
            _when(j + 2 < NTB, lambda: g_load(j + 2, slot).start())
            lend(_div(j + 1, 2), 1 - slot).start(priority=1)
            _wait(w1_load(j, slot), g_load(j + 1, 1 - slot))
            attention_out(j + 1)
            u = _mm_rows(w1s[slot], _from16(h_buf[...]), _mm_nt)
            u_acc[...] = _accumulate(j, u_acc[...], u)
            goT[:, _ds(j + 1, TB)] = gin[1 - slot].T
            ln23(j + 1, (u, 256, 128, 4), (u, 768, 128, 4))
            return 0

        lax.fori_loop(0, NTB - 1, mix_body, 0)
        w2_rows(0, FB, 0).start()
        w1_load(NTB - 1, 1).wait()
        u_acc[...] += _mm_rows(w1s[1], _from16(h_buf[...]), _mm_nt)
        _wait(*[lend(i, quarter) for i in range(NLEND)
                for quarter in range(2 if i < NLEND - 1 else 3)])

        k0 = math.sqrt(2.0 / math.pi)
        k1 = 0.044715

        def hidden(i, n, slot):
            gb = mod_row(5)
            for f0 in range(0, n, 128):
                k = min(128, n - f0)
                f = _ds(i * (FB // 128) + f0 // 128, 128).start
                dg = _mm_nt(_from16(w2r[slot, pl.ds(f0 // 16, k // 16)]), goT[...])
                u = u_acc[pl.ds(f, k), :] + _wide(_col(rows[B1:B1 + 1, pl.ds(f, k)]), D)
                u2 = u * u
                th = jnp.tanh(u * (k0 + (k0 * k1) * u2))
                cdf = 0.5 + 0.5 * th
                g = u * cdf
                dgelu = cdf + (0.5 * u) * (1.0 - th * th) * (k0 + (3.0 * k0 * k1) * u2)
                du = (dg * (dgelu * gb)).astype(bf16)
                p_buf[lent[0], pl.ds(_div(f, 16), k // 16)] = _to16(g * gb)
                p_buf[lent[1], pl.ds(_div(f, 16), k // 16)] = _to16(du)
                part = _ds(_div(f, D), D // 16)
                lanes = pl.ds(_ds(_div(_rem(f, D), 128), 128).start, k)
                p_buf[lent[2], part, :, lanes] = _to16(g.astype(bf16).T)
                du_t = du.T
                p_buf[lent[3], part, :, lanes] = _to16(du_t)
                rows[B1:B1 + 1, pl.ds(f, k)] = jnp.sum(du_t.astype(f32), axis=0, keepdims=True)

        full, left = divmod(F, FB)

        def hidden_body(i, _):
            slot = lax.rem(i, 2)
            _when(i + 1 < full, lambda: w2_rows(i + 1, FB, 1 - slot).start())
            _when(i + 1 == full,
                  lambda: _start(w2_rows(full, left, full % 2), c_wo, *w_loads(0, 0)))
            _when(i < NLEND - 1, lambda: lend(i, 2).start(priority=1))
            _when(i == (S // 2) // FB, lambda: _wait(*[lend(k, 2) for k in range(NLEND - 1)]))
            w2_rows(i, FB, slot).wait()
            hidden(i, FB, slot)
            return 0

        lax.fori_loop(0, full, hidden_body, 0)
        w2_rows(full, left, full % 2).wait()
        hidden(full, left, full % 2)

    def backward(goT, dw1s, dw2s, gacc, sums, dw_o, dkv_buf, o_sem):
        def stores(j, slot):
            tok = _ds(j, TB)
            return [cp(gin.at[slot], out_hbm.at[tok], o_sem.at[0, slot]),
                    cp(dw2s.at[slot], dw2_hbm.at[:, tok], o_sem.at[1, slot]),
                    cp(dw1s.at[slot], dw1T_hbm.at[:, tok], o_sem.at[2, slot])]

        def add_sum(step, i, x):
            sums[_ds(i, D), :] = _accumulate(step, sums[_ds(i, D), :], x)

        def tall(slot, f0, f1):
            return _from16(p_buf[slot, f0 // 16:f1 // 16])

        def wide(slot):
            return jnp.concatenate(
                [_from16(p_buf[slot, _ds(f0 // D, D // 16), :, 0:min(D, F - f0)])
                 for f0 in range(0, F, D)], axis=1)

        b1_buf[...] = rows[B1:B1 + 1, 0:F].reshape(F).astype(bf16)
        c_db1 = cp(b1_buf, db1_hbm, sem.at[0])
        c_db1.start()
        dkv_buf[...] = jnp.zeros_like(dkv_buf)
        col[2] = _col(mod_row(5))
        c_wo.wait()
        dw_o[...] = (wsq[...].astype(f32) * mod_row(2)).astype(bf16)

        def mlp_body(j, _):
            slot = lax.rem(j, 2)
            tok = _ds(j, TB)
            _when(j + 1 < NTB, lambda: _start(*w_loads(j + 1, 1 - slot)))
            _wait(*w_loads(j, slot))
            _when(j > 1, lambda: _wait(*stores(j - 2, slot)))
            y = _mm_rows(wide(lent[2]), _from16(w2_block(slot)[...])) + rows[B2:B2 + 1, tok]
            dh3 = _mm_rows(wide(lent[3]), w1s[slot])
            gt = goT[:, tok].astype(f32)
            gb = _wide(col[2], TB)
            rows[B2:B2 + 1, tok] = jnp.sum(gt * gb, axis=0, keepdims=True)
            xh2, r2, h3, r3 = ln23(j, (y, 0, 128, 4), (dh3, 0, 64, 4))
            h3 = h3.astype(bf16)
            dw1 = _mm_rows(tall(lent[1], 0, SPLIT), h3)
            dw1s[slot, 0:SPLIT] = dw1.astype(bf16)
            dw2 = _mm_rows(tall(lent[0], 0, F), goT[:, tok])
            dw2s[slot] = dw2.astype(bf16)
            gin[slot] = (xT[:, tok].astype(f32) + gb * y).astype(bf16).T
            add_sum(j, 2, _fold(gt * y))
            dx1 = []
            for i, (za, zb) in enumerate([((dw1, 0, 64, 4), (dw1, 384, 64, 4)),
                                          ((dw2, 0, 128, 4), (dw2, 512, 128, 4))]):
                t = slice(i * 128, (i + 1) * 128)
                dh2 = _ln_bwd(dh3[:, t], _from16(h_buf[:, :, t]).astype(f32), r3[:, t], za)
                add_sum(j + i, 0, dh2)
                add_sum(j + i, 1, dh2 * xh2[:, t])
                dx1.append(gt[:, t] + _ln_bwd(dh2 * col[1], xh2[:, t], r2[:, t], zb))
            dx1 = jnp.concatenate(dx1, axis=1).astype(bf16)
            xT[:, tok] = dx1
            ob = oT[:, tok]
            do = _mm(dw_o[...], dx1)
            gacc[...] = _accumulate(j, gacc[...], _mm_nt(ob, dx1))
            dw1s[slot, SPLIT:F] = _mm_rows(tall(lent[1], SPLIT, F), h3).astype(bf16)
            do = do.reshape(H, DH, TB) * l_buf[:, tok].reshape(H, 1, TB)
            l_buf[:, tok] = jnp.sum(do * ob.astype(f32).reshape(H, DH, TB), axis=1)
            oT[:, tok] = do.reshape(D, TB).astype(bf16)
            _start(*stores(j, slot))
            return 0

        lax.fori_loop(0, NTB, mlp_body, 0)

        qT = goT
        lead = DH * -(-UB // NQ)
        c_q = [cp(q_hbm.at[part], qT.at[part], sem.at[14 + i])
               for i, part in enumerate([pl.ds(D - lead, lead), pl.ds(0, D - lead)])]
        _start(*c_q)
        b2_buf[...] = rows[B2:B2 + 1, :].reshape(S).astype(bf16)
        g = gacc[...]
        dmod_buf[:, 2 * D:3 * D] = jnp.sum(g * wsq[...].astype(f32), axis=0, keepdims=True)
        dw_o[...] = (g * mod_row(2)).astype(bf16)
        for i in range(3):
            dmod_buf[:, (3 + i) * D:(4 + i) * D] = _row(sums[_ds(i, D), :])
        v_buf = sums
        for j in range(NQ):
            vt = pltpu.bitcast(kvT[DH // 2:DH, _ds(j, BQ)], bf16).astype(f32)
            v_buf[_ds(j, BQ // 2), :] = _rows_by_head_dim(vt)
        c_small = [cp(b2_buf, db2_hbm, sem.at[1]), cp(dw_o, dwo_hbm, sem.at[2]),
                   cp(wq_hbm, wsq, sem.at[3])]
        _start(*c_small)
        c_q[0].wait()

        def bwd_blocks(steps, slots, consumed=None):
            st = []
            for u, t in enumerate(steps):
                r, cq, hr = step_slices(t)
                st.append(dict(r=r, cq=cq, q=qT[r, cq], do=oT[r, cq], delta=l_buf[hr, cq],
                               m=None if slots else rows[max_slices(t)],
                               slot=slots[u] if slots else None))

            def load_p(s, c):
                return _from16(p_buf[s["slot"], pl.ds(c * (CK // 16), CK // 16)])

            def op_p(s, c):
                s["p", c] = jnp.exp2(_mm(head_rows(k_buf, c), s["q"]) - s["m"])

            def op_ds(s, c):
                dp = _mm(head_rows(v_buf, c), s["do"])
                p = load_p(s, c).astype(f32) if slots else s["p", c]
                s["ds", c] = (p * (dp - s["delta"])).astype(bf16)

            def op_dv(s, c):
                p = load_p(s, c) if slots else s["p", c].astype(bf16)
                dkv_buf[DH:2 * DH, pl.ds(c * CK, CK)] += _mm_nt(s["do"], p)

            def op_dk(s, c):
                dkv_buf[0:DH, pl.ds(c * CK, CK)] += _mm_nt(s["q"], s["ds", c])

            def op_dq(s, c):
                t = _mm(head_cols(0, c), s["ds", c])
                s["dq"] = t if c == 0 else s["dq"] + t
                if c == NC - 1:
                    qT[s["r"], s["cq"]] = (s["dq"] * QK_SCALE).astype(bf16)

            if slots:
                order = [(op_ds, 0), (op_dv, 0), (op_dk, 2), (op_dq, 2)]
            else:
                order = [(op_p, 0), (op_dv, 1), (op_ds, 1), (op_dk, 2), (op_dq, 2)]
            n = len(steps) * NC
            for g in range(n + 2):
                if g == n and consumed:
                    consumed()
                for op, lag in order:
                    if 0 <= g - lag < n:
                        op(st[(g - lag) // NC], (g - lag) % NC)

        def mlp_done():
            _wait(c_q[1], *stores(NTB - 2, 0), *stores(NTB - 1, 1))
            _start(*[repay(i) for i in range(NLEND)])

        def saved_blocks(first, count):
            def refill():
                for b in [first - u for u in range(1, count, 2)]:
                    _when(b >= NSLOT, lambda: p_read(b - NSLOT).start())
                ahead = first - count
                for b in [ahead - u for u in range(1, UB, 2)]:
                    _when((b >= 0) & (b < NHBM), lambda: p_read(b).wait())
                _when((ahead >= NHBM + NLEND - 1) & (ahead - UB < NHBM + NLEND - 1),
                      lambda: _wait(*[repay(i) for i in range(NLEND)]))

            bs = [first - u for u in range(count)]
            bwd_blocks([jnp.where(b < NSLOT, b, b + NREC) for b in bs], [_slot(b) for b in bs],
                       refill)

        def saved_body(i, _):
            _when(i == 1, mlp_done)
            saved_blocks(NSAVE - 1 - i * UB, UB)
            return 0

        lax.fori_loop(0, NSAVE // UB, saved_body, 0)
        if NSAVE % UB:
            saved_blocks(NSAVE % UB - 1, NSAVE % UB)

        _wait(c_db1, *c_small)
        c_in = [x_load(0, j) for j in range(NQ)] + [wmod_load(1, i) for i in range(6)]
        _start(*c_in)

        def rec_body(i, _):
            bwd_blocks([NSLOT + i * UR + u for u in range(UR)], None)
            return 0

        lax.fori_loop(0, NREC // UR, rec_body, 0)
        if NREC % UR:
            bwd_blocks([NSLOT + NREC - 1 - u for u in range(NREC % UR)], None)

        _wait(*c_in)
        cv = c_buf[...].astype(f32)
        sg = jax.nn.sigmoid(cv)
        col[0] = _col(mod_row(0))
        col[1] = _col(1.0 + mod_row(1))
        col[2] = _col((cv * sg).astype(bf16).astype(f32))
        h_buf[:, :, 0:128] = _to16(jnp.concatenate(
            [wkv[...].astype(f32), jnp.zeros((128 - 2 * DH, D), f32)], axis=0).T)
        dkv_buf[0:DH, :] = dkv_buf[0:DH, :] * LN2

        def dwmod_store(i):
            return cp(tile(3, i), dwmod_hbm.at[:, :, pl.ds(i * D, D)], sem.at[8])

        def dx_store(j):
            part = _ds(j, TB // 16)
            return cp(p_buf.at[5, part], dx_hbm.at[part], sem.at[4])

        def dwq_store(i, n):
            part = pl.ds(i * 128, n * 128)
            return cp(dw_o.at[part], dwq_hbm.at[part], sem.at[5])

        def mod_grad(i):
            tile(3, i)[...] = _to16(_wide(col[2], D) * dmod_buf[:, i * D:(i + 1) * D])

        def input_grad(j):
            tok = _ds(j, TB)
            kv_part = _mm(_from16(h_buf[:, :, 0:2 * DH]), dkv_buf[:, tok].astype(bf16))
            q_part = _mm_rows(wsq[...], qT[:, tok])
            return q_part + kv_part, q_part

        def norm_grad(j, pace=None):
            tok = _ds(j, TB)
            dh = gacc[:, 0:TB]
            xhat, h = modulated(_from16(p_buf[0, _ds(j, TB // 16)]).T, tok)
            oT[:, tok] = h
            for i in range(D // TB):
                gacc[_ds(i, 128), TB:] = _accumulate(
                    j, gacc[_ds(i, 128), TB:], _mm_nt(h[0:128], qT[_ds(i, TB), tok]))
            t = _mm_nt(dkv_buf[:, tok].astype(bf16), h)
            gacc[256:256 + 4 * DH, TB:] = _accumulate(
                j, gacc[256:256 + 4 * DH, TB:], jnp.concatenate([t[:, 0:TB], t[:, TB:]], axis=0))
            add_sum(j, 0, _fold(dh))
            add_sum(j, 1, _fold(dh * xhat))
            dx = xT[:, tok].astype(f32) + _ln_bwd(dh * _wide(col[1], TB), xhat,
                                                  rows[RSTD:RSTD + 1, tok], pace)
            p_buf[5, _ds(j, TB // 16)] = _to16(dx.astype(bf16).T)

        gacc[:, 0:TB] = input_grad(0)[0]
        for i in range(2, 6):
            mod_grad(i)
        _start(*[dwmod_store(i) for i in range(2, 6)])

        def tail_body(j, _):
            dh_next, dq_part = input_grad(j + 1)
            norm_grad(j, (dq_part, 0, 128, 2))
            gacc[:, 0:TB] = dh_next
            dx_store(j).start()
            return 0

        lax.fori_loop(0, NTB - 1, tail_body, 0)

        dsc = [0.0] * (D // 128)

        def weight_grad(i, mods):
            for n in range(D // 128):
                acc = 0.0
                for k in range(NQ):
                    acc = acc + _mm_nt(oT[_ds(i, 128), _ds(k, BQ)], qT[_ds(n, 128), _ds(k, BQ)])
                    if k < len(mods):
                        dm = jnp.broadcast_to(dmod_buf[:, _ds(mods[k], D)], (16, D))
                        w = _from16(tile(1, mods[k])[_ds(n, 8)])
                        dsc[n] = dsc[n] + _mm_nt(dm.astype(bf16), w)
                dw_o[_ds(i, 128), _ds(n, 128)] = acc.astype(bf16)

        norm_grad(NTB - 1)
        dw_o[0:128, :] = jnp.concatenate(
            [gacc[0:128, TB:], gacc[128:256, TB:]], axis=1).astype(bf16)
        wkv[...] = jnp.concatenate(
            [gacc[256:256 + 2 * DH, TB:], gacc[256 + 2 * DH:256 + 4 * DH, TB:]],
            axis=1).astype(bf16)
        weight_grad(1, (2, 3, 4))
        for i in range(2):
            dmod_buf[:, i * D:(i + 1) * D] = _row(sums[_ds(i, D), :])
            mod_grad(i)
        c_out = [cp(wkv.at[pl.ds(0, DH)], dwkT_hbm, sem.at[1]),
                 cp(wkv.at[pl.ds(DH, DH)], dwvT_hbm, sem.at[2]),
                 cp(c_buf, dc_hbm, sem.at[0]), dwq_store(0, 3), dwq_store(3, 1)]
        _start(dx_store(NTB - 1), dwmod_store(0), dwmod_store(1), *c_out[0:2])
        weight_grad(2, (5, 0, 1))
        c_buf[...] = (jnp.concatenate(dsc, axis=1)[0:1]
                      * (sg * (1.0 + cv * (1.0 - sg)))).astype(bf16)
        _start(*c_out[2:4])
        weight_grad(3, ())
        c_out[4].start()
        _wait(*c_out, *[dx_store(j) for j in range(NTB)], *[dwmod_store(i) for i in range(6)])

    def second_half(goT):
        pl.run_scoped(lambda *refs: mlp_hidden(goT, *refs), pltpu.VMEM((F, D), f32),
                pltpu.VMEM((2, FB // 16, 16, S), bf16), pltpu.SemaphoreType.DMA((2,)))
        pl.run_scoped(lambda *refs: backward(goT, *refs),
                pltpu.VMEM((2, F, TB), bf16), pltpu.VMEM((2, F, TB), bf16),
                pltpu.VMEM((D, D), f32), pltpu.VMEM((3 * D, 128), f32), pltpu.VMEM((D, D), bf16),
                pltpu.VMEM((2 * DH, S), f32),
                pltpu.SemaphoreType.DMA((3, 2)))

    pl.run_scoped(second_half, pltpu.VMEM((D, S), bf16))


@jax.jit
def pallas_adaLN_cond__grouped_kv_mqa__mixer_token_mlp__prompt_kernel(
    A_x: jax.Array,
    A_wq: jax.Array,
    A_wk: jax.Array,
    A_wv: jax.Array,
    A_wo: jax.Array,
    B_x: jax.Array,
    B_w1: jax.Array,
    B_b1: jax.Array,
    B_w2: jax.Array,
    B_b2: jax.Array,
    c: jax.Array,
    w_mod: jax.Array,
    grad_out: jax.Array,
):
    del B_x
    sds = jax.ShapeDtypeStruct
    p_block = (S // 16, 16, BQ)
    out_shape = [
        sds((S, D), bf16), sds((S // 16, 16, D), bf16), sds((D, D), bf16), sds((DH, D), bf16),
        sds((DH, D), bf16), sds((D, D), bf16), sds((F, S), bf16), sds((F,), bf16),
        sds((F, S), bf16), sds((S,), bf16), sds((1, D), bf16), sds((D // 16, 16, 6 * D), bf16),
        sds((NHBM,) + p_block, bf16), sds((NLEND, 3 * S // 64, 16, BQ), bf16), sds((D, S), bf16),
    ]
    hbm = pl.BlockSpec(memory_space=pl.ANY)
    outs = pl.pallas_call(
        _kernel,
        out_shape=out_shape,
        in_specs=[hbm] * 12,
        out_specs=[hbm] * len(out_shape),
        scratch_shapes=[
            pltpu.VMEM((NSLOT,) + p_block, bf16),
            pltpu.VMEM((D, S), bf16),
            pltpu.VMEM((D, S), bf16),
            pltpu.VMEM((S // 2, 128), f32),
            pltpu.VMEM((DH, S), u32),
            pltpu.VMEM((H, S), f32),
            pltpu.VMEM((8, S), f32),
            pltpu.VMEM((1, 6 * D), f32),
            pltpu.VMEM((1, 6 * D), f32),
            pltpu.VMEM((3, D, 128), f32),
            pltpu.VMEM((1, D), bf16),
            pltpu.VMEM((F,), bf16),
            pltpu.VMEM((S,), bf16),
            pltpu.VMEM((2, F, TB), bf16),
            pltpu.VMEM((D // 16, 16, TB), bf16),
            pltpu.VMEM((2, TB, D), bf16),
            pltpu.VMEM((D, D), bf16),
            pltpu.VMEM((2 * DH, D), bf16),
            pltpu.SemaphoreType.DMA((NSLOT,)),
            pltpu.SemaphoreType.DMA((3, 2)),
            pltpu.SemaphoreType.DMA((17,)),
        ],
        compiler_params=pltpu.CompilerParams(vmem_limit_bytes=128 * 2 ** 20,
                                             disable_semaphore_checks=True,
                                             disable_bounds_checks=True),
        name="adaln_mqa_mixer",
    )(A_x.reshape(S // 16, 16, D), A_wq, A_wk.T, A_wv.T, A_wo, B_w1.T, B_b1,
      B_w2.reshape(FT, 16, S), B_b2, c, w_mod.reshape(D // 16, 16, 6 * D),
      grad_out.reshape(S, D))
    out, dx, dwq, dwkT, dwvT, dwo, dw1T, db1, dw2, db2, dc, dwmod = outs[:12]
    return (out.reshape(1, S, D), dx.reshape(1, S, D), dwq, dwkT.T, dwvT.T, dwo, dw1T.T,
            db1, dw2, db2, dc, dwmod.reshape(D, 6 * D))
```

```python
import math

import jax
import jax.numpy as jnp
from jax import lax
import jax.experimental.pallas as pl
import jax.experimental.pallas.tpu as pltpu

f32 = jnp.float32
bf16 = jnp.bfloat16
u32 = jnp.uint32

S, D, H, DH, F = 2048, 512, 32, 16, 1376
EPS = 1e-5
QK_SCALE = DH ** -0.5
LOG2E = math.log2(math.e)
LN2 = math.log(2.0)

BQ = 512
CK = 128
NQ = S // BQ
NC = S // CK
NSTEP = H * NQ
UF = 4
HEAD = (1, 1)
TAIL = (1, 1)
UB = 8
UR = 4
NSLOT = 54
NSAVE = 116
NREC = NSTEP - NSAVE
NHBM = NSAVE - NSLOT
NLEND = 5
LAG = 2
DEP = 7
TB = 256
NTB = S // TB
FB = 256
FT = F // 16
SPLIT = 768
RING = UF * NC // 3
assert NTB == 2 * (NLEND - 1) and NREC <= 3 * NQ and RING > NC + LAG
assert NSAVE <= 3 * NSLOT and NSLOT % 2 == NSAVE % 2 == UB % 2 == 0
assert HEAD[0] == TAIL[-1] == 1 and sum(TAIL) >= 2
assert (NSTEP - sum(HEAD) - sum(TAIL)) % UF == 0


def _mm(a, b):
    return jnp.dot(a, b, preferred_element_type=f32)


def _mm_nt(a, b):
    return lax.dot_general(a, b, (((1,), (1,)), ((), ())), preferred_element_type=f32)


def _mm_rows(a, b, mm=_mm, rows=128):
    return jnp.concatenate([mm(a[i:i + rows], b) for i in range(0, a.shape[0], rows)], axis=0)


def _ds(i, n):
    if isinstance(i, int):
        return pl.ds(i * n, n)
    return pl.ds(pl.multiple_of(i * n, n), n)


def _div(i, n):
    return i // n if isinstance(i, int) else lax.div(i, jnp.int32(n))


def _rem(i, n):
    return i % n if isinstance(i, int) else lax.rem(i, jnp.int32(n))


def _slot(b):
    if isinstance(b, int):
        return b % NSLOT
    return b - jnp.where(b >= NSLOT, NSLOT, 0) - jnp.where(b >= 2 * NSLOT, NSLOT, 0)


def _when(cond, fn):
    if isinstance(cond, bool):
        if cond:
            fn()
    else:
        pl.when(cond)(fn)


def _start(*copies):
    for d in copies:
        d.start()


def _wait(*copies):
    for d in copies:
        d.wait()


def _after(v, z):
    return jnp.maximum(v, jnp.minimum(v, z))


def _accumulate(step, acc, x):
    return jnp.where(step == 0, 0.0, acc) + x


def _col(row):
    return jnp.broadcast_to(row, (128, row.shape[1])).T


def _wide(col, n):
    return jnp.concatenate([col] * (n // 128), axis=1)


def _fold(x):
    acc = x[:, 0:128]
    for i in range(1, x.shape[1] // 128):
        acc = acc + x[:, i * 128:(i + 1) * 128]
    return acc


def _row(partial):
    return jnp.sum(partial.T, axis=0, keepdims=True)


def _mean0(x):
    return jnp.sum(x, axis=0, keepdims=True) * (1.0 / x.shape[0])


def _paced(v, pace, n):
    if pace is None:
        return v
    z, first, step, groups = pace
    return jnp.concatenate(
        [jnp.broadcast_to(_after(v, z[i:i + 1, 0:v.shape[1]]), (n // groups, v.shape[1]))
         for i in range(first, first + step * groups, step)], axis=0)


def _ln(x, pace=None):
    mu = _mean0(x)
    xc = x - _paced(mu, pace, x.shape[0])
    r = lax.rsqrt(_mean0(xc * xc) + EPS)
    return xc * r, mu, r


def _ln_bwd(dy, xhat, r, pace=None):
    a, b = _mean0(dy), _mean0(dy * xhat)
    return r * (dy - _paced(a, pace, dy.shape[0]) - xhat * _paced(b, pace, dy.shape[0]))


def _rows_by_head_dim(xt):
    pad = jnp.concatenate([xt, jnp.zeros((128 - DH, xt.shape[1]), f32)], axis=0)
    return pltpu.bitcast(pad.T.astype(bf16), f32)


def _to16(v):
    return v.reshape(v.shape[0] // 16, 16, v.shape[1]).astype(bf16)


def _from16(v):
    return v.reshape(v.shape[0] * 16, v.shape[2])


def _kernel(x_hbm, wq_hbm, wkT_hbm, wvT_hbm, wo_hbm, w1T_hbm, b1_hbm, w2_hbm, b2_hbm,
            c_hbm, wmod_hbm, go_hbm,
            out_hbm, dx_hbm, dwq_hbm, dwkT_hbm, dwvT_hbm, dwo_hbm, dw1T_hbm, db1_hbm,
            dw2_hbm, db2_hbm, dc_hbm, dwmod_hbm, p_hbm, lent_hbm, q_hbm,
            p_buf, xT, oT, k_buf, kvT, l_buf, rows, mod_buf, dmod_buf, col, c_buf, b1_buf,
            b2_buf, w1s, h_buf, gin, wsq, wkv, p_sem, w_sem, sem):
    cp = pltpu.make_async_copy
    B1, B2, MU, RSTD, MAX = range(5)

    def mod_row(i):
        return mod_buf[:, i * D:(i + 1) * D]

    def step_slices(t):
        return _ds(_div(t, NQ), DH), _ds(_rem(t, NQ), BQ), pl.ds(_div(t, NQ), 1)

    def max_slices(t):
        kept = (t >= NSLOT) & (t < NSLOT + NREC)
        return pl.ds(jnp.where(kept, MAX + _div(t - NSLOT, NQ), 7), 1), _ds(_rem(t, NQ), BQ)

    def p_write(b):
        return cp(p_buf.at[_slot(b)], p_hbm.at[b], p_sem.at[_slot(b)])

    def p_read(b):
        return cp(p_hbm.at[pl.ds(b, 2)], p_buf.at[pl.ds(_slot(b), 2)], p_sem.at[_slot(b)])

    def lend(i, quarter):
        part, slot = _ds(quarter, S // 64), _slot(NHBM + i)
        return cp(p_buf.at[slot, part], lent_hbm.at[i, part], p_sem.at[slot])

    def repay(i):
        slot = _slot(NHBM + i)
        return cp(lent_hbm.at[i], p_buf.at[slot, pl.ds(0, 3 * S // 64)], p_sem.at[slot])

    def tile(slot, i):
        return p_buf.at[slot + _div(i, 4), _ds(_rem(i, 4), D // 16)]

    def x_load(slot, j):
        return cp(x_hbm.at[_ds(j, BQ // 16)], tile(slot, j), sem.at[4 + j])

    def wmod_load(slot, i):
        return cp(wmod_hbm.at[:, :, pl.ds(i * D, D)], tile(slot, i), sem.at[8 + i])

    def w1_load(j, slot):
        return cp(w1T_hbm.at[:, _ds(j, TB)], w1s.at[slot], w_sem.at[1, slot])

    def g_load(j, slot):
        return cp(go_hbm.at[_ds(j, TB)], gin.at[slot], w_sem.at[2, slot])

    def head_rows(buf, c):
        return pltpu.bitcast(buf[pl.ds(c * (CK // 2), CK // 2), 0:DH], bf16)

    def head_cols(i, c):
        return pltpu.bitcast(kvT[i * (DH // 2):(i + 1) * (DH // 2), pl.ds(c * CK, CK)], bf16)

    def modulated(x, tok):
        xhat = (x.astype(f32) - rows[MU:MU + 1, tok]) * rows[RSTD:RSTD + 1, tok]
        n = x.shape[1]
        return xhat, (xhat * _wide(col[1], n) + _wide(col[0], n)).astype(bf16)

    def attention_out(j):
        tok = _ds(j, TB)
        a = _mm(wsq[...], oT[:, tok])
        xT[:, tok] = (xT[:, tok].astype(f32) + _wide(col[2], TB) * a).astype(bf16)

    def ln23(j, za=None, zb=None):
        xh2, _, r2 = _ln(xT[:, _ds(j, TB)].astype(f32), za)
        h3, _, r3 = _ln(xh2 * _wide(col[1], TB) + _wide(col[0], TB), zb)
        h_buf[...] = _to16(h3)
        return xh2, r2, h3, r3

    c_wo = cp(wo_hbm, wsq, sem.at[14])

    def first_half(s_buf, wqT, h1):
        c_c = cp(c_hbm, c_buf, sem.at[0])
        c_k = cp(wkT_hbm, wkv.at[pl.ds(0, DH)], sem.at[1])
        c_v = cp(wvT_hbm, wkv.at[pl.ds(DH, DH)], sem.at[2])
        c_q = cp(wq_hbm, wsq, sem.at[3])
        c_m = [wmod_load(NSLOT - 3, i) for i in range(6)]
        c_b = [cp(b1_hbm, b1_buf, sem.at[15]), cp(b2_hbm, b2_buf, sem.at[16])]
        c_x = [x_load(NSLOT - 1, j) for j in range(NQ)]
        _start(c_c, *c_m[:2], c_x[0], c_k, c_v, c_q, *c_x[1:], *c_m[2:], *c_b, g_load(0, 0),
               w1_load(0, 0))

        def mod_part(i, lanes):
            cv = c_buf[...].astype(f32)
            sc = jnp.broadcast_to(cv * jax.nn.sigmoid(cv), (16, D)).astype(bf16)
            w = _from16(tile(NSLOT - 3, i)[:, :, lanes])
            mod_buf[:, pl.ds(i * D + lanes.start, lanes.size)] = _mm(sc, w)[0:1]

        _wait(c_c, *c_m[:2])
        mod_part(0, pl.ds(0, D))
        mod_part(1, pl.ds(0, D))
        col[0] = _col(mod_row(0))
        col[1] = _col(1.0 + mod_row(1))

        def normalize(j, q=None):
            for i in range(BQ // 128):
                tok = _ds(j * (BQ // 128) + i, 128)
                xt = _from16(tile(NSLOT - 1, j)[_ds(i, 8)]).T
                xT[:, tok] = xt
                xhat, rows[MU:MU + 1, tok], rows[RSTD:RSTD + 1, tok] = _ln(
                    xt.astype(f32), None if q is None else (q, 96 * i, 32, 4))
                h1[:, _ds(i, 128)] = (xhat * col[1] + col[0]).astype(bf16)

        def project(j):
            tok = _ds(j, BQ)
            kv = _mm(wkv[...], h1[...])
            kvT[:, tok] = pltpu.bitcast(kv.astype(bf16), u32)
            k_buf[_ds(j, BQ // 2), :] = _rows_by_head_dim(kv[0:DH])
            q = _mm_rows(wqT[...], h1[...], rows=64)
            oT[:, tok] = (q * (QK_SCALE * LOG2E)).astype(bf16)
            return q

        def project_body(j, _):
            x_load(NSLOT - 1, j + 1).wait()
            normalize(j + 1, project(j))
            return 0

        c_x[0].wait()
        normalize(0)
        _wait(c_k, c_v, c_q)
        wqT[...] = wsq[...].T
        c_wo.start()
        lax.fori_loop(0, NQ - 1, project_body, 0)
        project(NQ - 1)
        c_qo = [cp(oT.at[:, _ds(j, BQ)], q_hbm.at[:, _ds(j, BQ)], sem.at[j]) for j in range(NQ)]
        _start(*c_qo)
        _wait(*c_m[2:])

        def s_rows(phase, c):
            g = (phase % UF) * NC + c
            return pl.ds((g - min(g // RING, 2) * RING) * CK, CK)

        def s_chunk(q, phase, c, mx, hist):
            s = _mm(head_rows(k_buf, c), q)
            s_buf[s_rows(phase, c), :] = s
            for half in (s[:CK // 2], s[CK // 2:]):
                part = jnp.max(half.reshape(CK // 16, 8, BQ), axis=0)
                mx = part if mx is None else jnp.maximum(mx, part)
                hist.append(mx)
            return mx

        def load_q(t):
            r, cq, _ = step_slices(t)
            return oT[r, cq]

        def saved_index(t):
            if isinstance(t, int):
                return t if t < NSLOT else max(t - NREC, NSLOT)
            return jnp.where(t < NSLOT, t, jnp.maximum(t - NREC, NSLOT))

        def release_slots(t0, count):
            for t in [t0 + u for u in range(count)]:
                b = saved_index(t)
                saved = (t < NSLOT) | (t >= NSLOT + NREC)
                _when(saved & (b < NHBM), lambda: p_write(b).start(priority=1))

        def claim_slots(t0, count):
            slots = []
            for t in [t0 + u for u in range(count)]:
                b = saved_index(t)
                _when((t == NSLOT) | (t > NSLOT + NREC), lambda: p_write(b - NSLOT).wait())
                slots.append(_slot(b))
            return slots

        def blocks(t0, phase, slots, m, mx):
            qs, hist = {}, []
            for u, slot in enumerate(slots):
                r, cq, hr = step_slices(t0 + u)
                m8 = jnp.broadcast_to(m, (8, BQ))
                m_next = l = o = None
                for c in range(NC):
                    du, sc = divmod(u * NC + c + NC + LAG, NC)
                    ahead = not (isinstance(t0, int) and t0 + du >= NSTEP)
                    if ahead:
                        if du not in qs:
                            qs[du] = load_q(t0 + du)
                        mx = s_chunk(qs[du], phase + du, sc, None if sc == 0 else mx, hist)
                        if sc == NC - 1:
                            m_next = jnp.max(mx, axis=0, keepdims=True)
                    k = 2 * (u * NC + c) + 1 - DEP
                    mc = _after(m8, hist[k]) if k >= 0 else m8
                    p = jnp.exp2(s_buf[s_rows(phase + u, c), :]
                                 - jnp.concatenate([mc] * (CK // 8), axis=0))
                    lp = p[CK - 8:CK]
                    for i in reversed(range(CK // 8 - 1)):
                        lp = lp + p[i * 8:(i + 1) * 8]
                    l = lp if l is None else l + lp
                    p_buf[slot, pl.ds(c * (CK // 16), CK // 16)] = _to16(p)
                    op = _mm(head_cols(1, c), p.astype(bf16))
                    o = op if o is None else o + op
                    if not ahead:
                        hist += [op[0:8], op[8:16]]
                linv = 1.0 / jnp.sum(l, axis=0, keepdims=True)
                if isinstance(t0, int) and t0 + u == 0:
                    c_qo[0].wait()
                oT[r, cq] = (o * linv).astype(bf16)
                rows[max_slices(t0 + u)] = m
                l_buf[hr, cq] = linv
                m = m_next
            return m, mx

        q0, mx = load_q(0), None
        for c in range(NC):
            mx = s_chunk(q0, 0, c, mx, [])
            mod_part(2 + c // 4, pl.ds((c % 4) * 128, 128))
        m = jnp.max(mx, axis=0, keepdims=True)
        q1, mx = load_q(1), None
        for c in range(LAG):
            mx = s_chunk(q1, 1, c, mx, [])
        t0 = 0
        for i, n in enumerate(HEAD):
            m, mx = blocks(t0, t0, claim_slots(t0, n), m, mx)
            release_slots(t0, n)
            if i == 0:
                _wait(*c_qo[1:], c_wo, *c_b)
            t0 += n
        first, trips = t0, (NSTEP - sum(HEAD) - sum(TAIL)) // UF

        def body(it, carry):
            t = first + it * UF
            carry = blocks(t, first, claim_slots(t, UF), *carry)
            release_slots(t, UF)
            return carry

        m, mx = lax.fori_loop(0, trips, body, (m, mx))
        t0 = first + trips * UF
        for i, n in enumerate(TAIL):
            slots = claim_slots(t0, n)
            if i == 0:
                col[0] = _col(mod_row(3))
                col[1] = _col(1.0 + mod_row(4))
                col[2] = _col(mod_row(2))
                wsq[...] = wsq[...].T
                rows[B1:B1 + 1, 0:F] = b1_buf[...].astype(f32).reshape(1, F)
                rows[B2:B2 + 1, :] = b2_buf[...].astype(f32).reshape(1, S)
            if i == len(TAIL) - 1:
                _start(*[lend(NLEND - 1, quarter) for quarter in range(3)], g_load(1, 1))
                attention_out(0)
                ln23(0)
            m, mx = blocks(t0, t0, slots, m, mx)
            t0 += n

    pl.run_scoped(first_half, pltpu.VMEM(((UF * NC - 2 * RING) * CK, BQ), f32),
            pltpu.VMEM((D, D), bf16), pltpu.VMEM((D, BQ), bf16))

    lent = [(NHBM + i) % NSLOT for i in range(NLEND)]

    def w2_block(slot):
        return p_buf.at[lent[4], pl.ds(0, FT), :, _ds(slot, TB)]

    def w_loads(j, slot):
        return [cp(w2_hbm.at[:, :, _ds(j, TB)], w2_block(slot), w_sem.at[0, slot]),
                w1_load(j, slot)]

    def mlp_hidden(goT, u_acc, w2r, r_sem):
        def w2_rows(i, n, slot):
            return cp(w2_hbm.at[pl.ds(i * (FB // 16), n // 16)],
                      w2r.at[slot, pl.ds(0, n // 16)], r_sem.at[slot])

        g_load(0, 0).wait()
        lend(0, 0).start(priority=1)
        goT[:, 0:TB] = gin[0].T

        def mix_body(j, _):
            slot = lax.rem(j, 2)
            w1_load(j + 1, 1 - slot).start()
            _when(j + 2 < NTB, lambda: g_load(j + 2, slot).start())
            lend(_div(j + 1, 2), 1 - slot).start(priority=1)
            _wait(w1_load(j, slot), g_load(j + 1, 1 - slot))
            attention_out(j + 1)
            u = _mm_rows(w1s[slot], _from16(h_buf[...]), _mm_nt)
            u_acc[...] = _accumulate(j, u_acc[...], u)
            goT[:, _ds(j + 1, TB)] = gin[1 - slot].T
            ln23(j + 1, (u, 256, 128, 4), (u, 768, 128, 4))
            return 0

        lax.fori_loop(0, NTB - 1, mix_body, 0)
        w2_rows(0, FB, 0).start()
        w1_load(NTB - 1, 1).wait()
        u_acc[...] += _mm_rows(w1s[1], _from16(h_buf[...]), _mm_nt)
        _wait(*[lend(i, quarter) for i in range(NLEND)
                for quarter in range(2 if i < NLEND - 1 else 3)])

        k0 = math.sqrt(2.0 / math.pi)
        k1 = 0.044715

        def hidden(i, n, slot):
            gb = mod_row(5)
            for f0 in range(0, n, 128):
                k = min(128, n - f0)
                f = _ds(i * (FB // 128) + f0 // 128, 128).start
                dg = _mm_nt(_from16(w2r[slot, pl.ds(f0 // 16, k // 16)]), goT[...])
                u = u_acc[pl.ds(f, k), :] + _wide(_col(rows[B1:B1 + 1, pl.ds(f, k)]), D)
                u2 = u * u
                th = jnp.tanh(u * (k0 + (k0 * k1) * u2))
                cdf = 0.5 + 0.5 * th
                g = u * cdf
                dgelu = cdf + (0.5 * u) * (1.0 - th * th) * (k0 + (3.0 * k0 * k1) * u2)
                du = (dg * (dgelu * gb)).astype(bf16)
                p_buf[lent[0], pl.ds(_div(f, 16), k // 16)] = _to16(g * gb)
                p_buf[lent[1], pl.ds(_div(f, 16), k // 16)] = _to16(du)
                part = _ds(_div(f, D), D // 16)
                lanes = pl.ds(_ds(_div(_rem(f, D), 128), 128).start, k)
                p_buf[lent[2], part, :, lanes] = _to16(g.astype(bf16).T)
                du_t = du.T
                p_buf[lent[3], part, :, lanes] = _to16(du_t)
                rows[B1:B1 + 1, pl.ds(f, k)] = jnp.sum(du_t.astype(f32), axis=0, keepdims=True)

        full, left = divmod(F, FB)

        def hidden_body(i, _):
            slot = lax.rem(i, 2)
            _when(i + 1 < full, lambda: w2_rows(i + 1, FB, 1 - slot).start())
            _when(i + 1 == full,
                  lambda: _start(w2_rows(full, left, full % 2), c_wo, *w_loads(0, 0)))
            _when(i < NLEND - 1, lambda: lend(i, 2).start(priority=1))
            _when(i == (S // 2) // FB, lambda: _wait(*[lend(k, 2) for k in range(NLEND - 1)]))
            w2_rows(i, FB, slot).wait()
            hidden(i, FB, slot)
            return 0

        lax.fori_loop(0, full, hidden_body, 0)
        w2_rows(full, left, full % 2).wait()
        hidden(full, left, full % 2)

    def backward(goT, dw1s, dw2s, gacc, sums, dw_o, dkv_buf, o_sem):
        def stores(j, slot):
            tok = _ds(j, TB)
            return [cp(gin.at[slot], out_hbm.at[tok], o_sem.at[0, slot]),
                    cp(dw2s.at[slot], dw2_hbm.at[:, tok], o_sem.at[1, slot]),
                    cp(dw1s.at[slot], dw1T_hbm.at[:, tok], o_sem.at[2, slot])]

        def add_sum(step, i, x):
            sums[_ds(i, D), :] = _accumulate(step, sums[_ds(i, D), :], x)

        def tall(slot, f0, f1):
            return _from16(p_buf[slot, f0 // 16:f1 // 16])

        def wide(slot):
            return jnp.concatenate(
                [_from16(p_buf[slot, _ds(f0 // D, D // 16), :, 0:min(D, F - f0)])
                 for f0 in range(0, F, D)], axis=1)

        b1_buf[...] = rows[B1:B1 + 1, 0:F].reshape(F).astype(bf16)
        c_db1 = cp(b1_buf, db1_hbm, sem.at[0])
        c_db1.start()
        dkv_buf[...] = jnp.zeros_like(dkv_buf)
        col[2] = _col(mod_row(5))
        c_wo.wait()
        dw_o[...] = (wsq[...].astype(f32) * mod_row(2)).astype(bf16)

        def mlp_body(j, _):
            slot = lax.rem(j, 2)
            tok = _ds(j, TB)
            _when(j + 1 < NTB, lambda: _start(*w_loads(j + 1, 1 - slot)))
            _wait(*w_loads(j, slot))
            _when(j > 1, lambda: _wait(*stores(j - 2, slot)))
            y = _mm_rows(wide(lent[2]), _from16(w2_block(slot)[...])) + rows[B2:B2 + 1, tok]
            dh3 = _mm_rows(wide(lent[3]), w1s[slot])
            gt = goT[:, tok].astype(f32)
            gb = _wide(col[2], TB)
            rows[B2:B2 + 1, tok] = jnp.sum(gt * gb, axis=0, keepdims=True)
            xh2, r2, h3, r3 = ln23(j, (y, 0, 128, 4), (dh3, 0, 64, 4))
            h3 = h3.astype(bf16)
            dw1 = _mm_rows(tall(lent[1], 0, SPLIT), h3)
            dw1s[slot, 0:SPLIT] = dw1.astype(bf16)
            dw2 = _mm_rows(tall(lent[0], 0, F), goT[:, tok])
            dw2s[slot] = dw2.astype(bf16)
            gin[slot] = (xT[:, tok].astype(f32) + gb * y).astype(bf16).T
            add_sum(j, 2, _fold(gt * y))
            dx1 = []
            for i, (za, zb) in enumerate([((dw1, 0, 64, 4), (dw1, 384, 64, 4)),
                                          ((dw2, 0, 128, 4), (dw2, 512, 128, 4))]):
                t = slice(i * 128, (i + 1) * 128)
                dh2 = _ln_bwd(dh3[:, t], _from16(h_buf[:, :, t]).astype(f32), r3[:, t], za)
                add_sum(j + i, 0, dh2)
                add_sum(j + i, 1, dh2 * xh2[:, t])
                dx1.append(gt[:, t] + _ln_bwd(dh2 * col[1], xh2[:, t], r2[:, t], zb))
            dx1 = jnp.concatenate(dx1, axis=1).astype(bf16)
            xT[:, tok] = dx1
            ob = oT[:, tok]
            do = _mm(dw_o[...], dx1)
            gacc[...] = _accumulate(j, gacc[...], _mm_nt(ob, dx1))
            dw1s[slot, SPLIT:F] = _mm_rows(tall(lent[1], SPLIT, F), h3).astype(bf16)
            do = do.reshape(H, DH, TB) * l_buf[:, tok].reshape(H, 1, TB)
            l_buf[:, tok] = jnp.sum(do * ob.astype(f32).reshape(H, DH, TB), axis=1)
            oT[:, tok] = do.reshape(D, TB).astype(bf16)
            _start(*stores(j, slot))
            return 0

        lax.fori_loop(0, NTB, mlp_body, 0)

        qT = goT
        lead = DH * -(-UB // NQ)
        c_q = [cp(q_hbm.at[part], qT.at[part], sem.at[14 + i])
               for i, part in enumerate([pl.ds(D - lead, lead), pl.ds(0, D - lead)])]
        _start(*c_q)
        b2_buf[...] = rows[B2:B2 + 1, :].reshape(S).astype(bf16)
        g = gacc[...]
        dmod_buf[:, 2 * D:3 * D] = jnp.sum(g * wsq[...].astype(f32), axis=0, keepdims=True)
        dw_o[...] = (g * mod_row(2)).astype(bf16)
        for i in range(3):
            dmod_buf[:, (3 + i) * D:(4 + i) * D] = _row(sums[_ds(i, D), :])
        v_buf = sums
        for j in range(NQ):
            vt = pltpu.bitcast(kvT[DH // 2:DH, _ds(j, BQ)], bf16).astype(f32)
            v_buf[_ds(j, BQ // 2), :] = _rows_by_head_dim(vt)
        c_small = [cp(b2_buf, db2_hbm, sem.at[1]), cp(dw_o, dwo_hbm, sem.at[2]),
                   cp(wq_hbm, wsq, sem.at[3])]
        _start(*c_small)
        c_q[0].wait()

        def bwd_blocks(steps, slots):
            st = []
            for u, t in enumerate(steps):
                r, cq, hr = step_slices(t)
                st.append(dict(r=r, cq=cq, q=qT[r, cq], do=oT[r, cq], delta=l_buf[hr, cq],
                               m=None if slots else rows[max_slices(t)],
                               slot=slots[u] if slots else None))

            def load_p(s, c):
                return _from16(p_buf[s["slot"], pl.ds(c * (CK // 16), CK // 16)])

            def op_p(s, c):
                s["p", c] = jnp.exp2(_mm(head_rows(k_buf, c), s["q"]) - s["m"])

            def op_ds(s, c):
                dp = _mm(head_rows(v_buf, c), s["do"])
                p = load_p(s, c).astype(f32) if slots else s["p", c]
                s["ds", c] = (p * (dp - s["delta"])).astype(bf16)

            def op_dv(s, c):
                p = load_p(s, c) if slots else s["p", c].astype(bf16)
                dkv_buf[DH:2 * DH, pl.ds(c * CK, CK)] += _mm_nt(s["do"], p)

            def op_dk(s, c):
                dkv_buf[0:DH, pl.ds(c * CK, CK)] += _mm_nt(s["q"], s["ds", c])

            def op_dq(s, c):
                t = _mm(head_cols(0, c), s["ds", c])
                s["dq"] = t if c == 0 else s["dq"] + t
                if c == NC - 1:
                    qT[s["r"], s["cq"]] = (s["dq"] * QK_SCALE).astype(bf16)

            if slots:
                order = [(op_ds, 0), (op_dv, 0), (op_dk, 2), (op_dq, 2)]
            else:
                order = [(op_p, 0), (op_dv, 2), (op_ds, 1), (op_dk, 2), (op_dq, 2)]
            n = len(steps) * NC
            for g in range(n + 2):
                for op, lag in order:
                    if 0 <= g - lag < n:
                        op(st[(g - lag) // NC], (g - lag) % NC)

        def mlp_done():
            _wait(c_q[1], *stores(NTB - 2, 0), *stores(NTB - 1, 1))
            _start(*[repay(i) for i in range(NLEND)])

        def saved_blocks(first, count):
            bs = [first - u for u in range(count)]
            bwd_blocks([jnp.where(b < NSLOT, b, b + NREC) for b in bs], [_slot(b) for b in bs])
            for b in bs[1::2]:
                _when(b >= NSLOT, lambda: p_read(b - NSLOT).start())
            ahead = first - count
            for b in [ahead - u for u in range(1, UB, 2)]:
                _when((b >= 0) & (b < NHBM), lambda: p_read(b).wait())
            _when((ahead >= NHBM + NLEND - 1) & (ahead - UB < NHBM + NLEND - 1),
                  lambda: _wait(*[repay(i) for i in range(NLEND)]))

        def saved_body(i, _):
            saved_blocks(NSAVE - 1 - i * UB, UB)
            _when(i == 0, mlp_done)
            return 0

        lax.fori_loop(0, NSAVE // UB, saved_body, 0)
        if NSAVE % UB:
            saved_blocks(NSAVE % UB - 1, NSAVE % UB)

        _wait(c_db1, *c_small)
        c_in = [x_load(0, j) for j in range(NQ)] + [wmod_load(1, i) for i in range(6)]
        _start(*c_in)

        def rec_body(i, _):
            bwd_blocks([NSLOT + i * UR + u for u in range(UR)], None)
            return 0

        lax.fori_loop(0, NREC // UR, rec_body, 0)
        if NREC % UR:
            bwd_blocks([NSLOT + NREC - 1 - u for u in range(NREC % UR)], None)

        _wait(*c_in)
        cv = c_buf[...].astype(f32)
        sg = jax.nn.sigmoid(cv)
        col[0] = _col(mod_row(0))
        col[1] = _col(1.0 + mod_row(1))
        col[2] = _col((cv * sg).astype(bf16).astype(f32))
        h_buf[:, :, 0:128] = _to16(jnp.concatenate(
            [wkv[...].astype(f32), jnp.zeros((128 - 2 * DH, D), f32)], axis=0).T)
        dkv_buf[0:DH, :] = dkv_buf[0:DH, :] * LN2

        def dwmod_store(i):
            return cp(tile(3, i), dwmod_hbm.at[:, :, pl.ds(i * D, D)], sem.at[8])

        def dx_store(j):
            part = _ds(j, TB // 16)
            return cp(p_buf.at[5, part], dx_hbm.at[part], sem.at[4])

        def dwq_store(i, n):
            part = pl.ds(i * 128, n * 128)
            return cp(dw_o.at[part], dwq_hbm.at[part], sem.at[5])

        def mod_grad(i):
            tile(3, i)[...] = _to16(_wide(col[2], D) * dmod_buf[:, i * D:(i + 1) * D])

        def input_grad(j):
            tok = _ds(j, TB)
            kv_part = _mm(_from16(h_buf[:, :, 0:2 * DH]), dkv_buf[:, tok].astype(bf16))
            q_part = _mm_rows(wsq[...], qT[:, tok])
            return q_part + kv_part, q_part

        def norm_grad(j, pace=None):
            tok = _ds(j, TB)
            dh = gacc[:, 0:TB]
            xhat, h = modulated(_from16(p_buf[0, _ds(j, TB // 16)]).T, tok)
            oT[:, tok] = h
            for i in range(D // TB):
                gacc[_ds(i, 128), TB:] = _accumulate(
                    j, gacc[_ds(i, 128), TB:], _mm_nt(h[0:128], qT[_ds(i, TB), tok]))
            t = _mm_nt(dkv_buf[:, tok].astype(bf16), h)
            gacc[256:256 + 4 * DH, TB:] = _accumulate(
                j, gacc[256:256 + 4 * DH, TB:], jnp.concatenate([t[:, 0:TB], t[:, TB:]], axis=0))
            add_sum(j, 0, _fold(dh))
            add_sum(j, 1, _fold(dh * xhat))
            dx = xT[:, tok].astype(f32) + _ln_bwd(dh * _wide(col[1], TB), xhat,
                                                  rows[RSTD:RSTD + 1, tok], pace)
            p_buf[5, _ds(j, TB // 16)] = _to16(dx.astype(bf16).T)

        gacc[:, 0:TB] = input_grad(0)[0]
        for i in range(2, 6):
            mod_grad(i)
        _start(*[dwmod_store(i) for i in range(2, 6)])

        def tail_body(j, _):
            dh_next, dq_part = input_grad(j + 1)
            norm_grad(j, (dq_part, 0, 128, 2))
            gacc[:, 0:TB] = dh_next
            dx_store(j).start()
            return 0

        lax.fori_loop(0, NTB - 1, tail_body, 0)

        dsc = [0.0] * (D // 128)

        def weight_grad(i, mods):
            for n in range(D // 128):
                acc = 0.0
                for k in range(NQ):
                    acc = acc + _mm_nt(oT[_ds(i, 128), _ds(k, BQ)], qT[_ds(n, 128), _ds(k, BQ)])
                    if k < len(mods):
                        dm = jnp.broadcast_to(dmod_buf[:, _ds(mods[k], D)], (16, D))
                        w = _from16(tile(1, mods[k])[_ds(n, 8)])
                        dsc[n] = dsc[n] + _mm_nt(dm.astype(bf16), w)
                dw_o[_ds(i, 128), _ds(n, 128)] = acc.astype(bf16)

        norm_grad(NTB - 1)
        dw_o[0:128, :] = jnp.concatenate(
            [gacc[0:128, TB:], gacc[128:256, TB:]], axis=1).astype(bf16)
        wkv[...] = jnp.concatenate(
            [gacc[256:256 + 2 * DH, TB:], gacc[256 + 2 * DH:256 + 4 * DH, TB:]],
            axis=1).astype(bf16)
        weight_grad(1, (2, 3, 4))
        for i in range(2):
            dmod_buf[:, i * D:(i + 1) * D] = _row(sums[_ds(i, D), :])
            mod_grad(i)
        c_out = [cp(wkv.at[pl.ds(0, DH)], dwkT_hbm, sem.at[1]),
                 cp(wkv.at[pl.ds(DH, DH)], dwvT_hbm, sem.at[2]),
                 cp(c_buf, dc_hbm, sem.at[0]), dwq_store(0, 3), dwq_store(3, 1)]
        _start(dx_store(NTB - 1), dwmod_store(0), dwmod_store(1), *c_out[0:2])
        weight_grad(2, (5, 0, 1))
        c_buf[...] = (jnp.concatenate(dsc, axis=1)[0:1]
                      * (sg * (1.0 + cv * (1.0 - sg)))).astype(bf16)
        _start(*c_out[2:4])
        weight_grad(3, ())
        c_out[4].start()
        _wait(*c_out, *[dx_store(j) for j in range(NTB)], *[dwmod_store(i) for i in range(6)])

    def second_half(goT):
        pl.run_scoped(lambda *refs: mlp_hidden(goT, *refs), pltpu.VMEM((F, D), f32),
                pltpu.VMEM((2, FB // 16, 16, S), bf16), pltpu.SemaphoreType.DMA((2,)))
        pl.run_scoped(lambda *refs: backward(goT, *refs),
                pltpu.VMEM((2, F, TB), bf16), pltpu.VMEM((2, F, TB), bf16),
                pltpu.VMEM((D, D), f32), pltpu.VMEM((3 * D, 128), f32), pltpu.VMEM((D, D), bf16),
                pltpu.VMEM((2 * DH, S), f32),
                pltpu.SemaphoreType.DMA((3, 2)))

    pl.run_scoped(second_half, pltpu.VMEM((D, S), bf16))


@jax.jit
def pallas_adaLN_cond__grouped_kv_mqa__mixer_token_mlp__prompt_kernel(
    A_x: jax.Array,
    A_wq: jax.Array,
    A_wk: jax.Array,
    A_wv: jax.Array,
    A_wo: jax.Array,
    B_x: jax.Array,
    B_w1: jax.Array,
    B_b1: jax.Array,
    B_w2: jax.Array,
    B_b2: jax.Array,
    c: jax.Array,
    w_mod: jax.Array,
    grad_out: jax.Array,
):
    del B_x
    sds = jax.ShapeDtypeStruct
    p_block = (S // 16, 16, BQ)
    out_shape = [
        sds((S, D), bf16), sds((S // 16, 16, D), bf16), sds((D, D), bf16), sds((DH, D), bf16),
        sds((DH, D), bf16), sds((D, D), bf16), sds((F, S), bf16), sds((F,), bf16),
        sds((F, S), bf16), sds((S,), bf16), sds((1, D), bf16), sds((D // 16, 16, 6 * D), bf16),
        sds((NHBM,) + p_block, bf16), sds((NLEND, 3 * S // 64, 16, BQ), bf16), sds((D, S), bf16),
    ]
    hbm = pl.BlockSpec(memory_space=pl.ANY)
    outs = pl.pallas_call(
        _kernel,
        out_shape=out_shape,
        in_specs=[hbm] * 12,
        out_specs=[hbm] * len(out_shape),
        scratch_shapes=[
            pltpu.VMEM((NSLOT,) + p_block, bf16),
            pltpu.VMEM((D, S), bf16),
            pltpu.VMEM((D, S), bf16),
            pltpu.VMEM((S // 2, 128), f32),
            pltpu.VMEM((DH, S), u32),
            pltpu.VMEM((H, S), f32),
            pltpu.VMEM((8, S), f32),
            pltpu.VMEM((1, 6 * D), f32),
            pltpu.VMEM((1, 6 * D), f32),
            pltpu.VMEM((3, D, 128), f32),
            pltpu.VMEM((1, D), bf16),
            pltpu.VMEM((F,), bf16),
            pltpu.VMEM((S,), bf16),
            pltpu.VMEM((2, F, TB), bf16),
            pltpu.VMEM((D // 16, 16, TB), bf16),
            pltpu.VMEM((2, TB, D), bf16),
            pltpu.VMEM((D, D), bf16),
            pltpu.VMEM((2 * DH, D), bf16),
            pltpu.SemaphoreType.DMA((NSLOT,)),
            pltpu.SemaphoreType.DMA((3, 2)),
            pltpu.SemaphoreType.DMA((17,)),
        ],
        compiler_params=pltpu.CompilerParams(vmem_limit_bytes=128 * 2 ** 20,
                                             disable_semaphore_checks=True,
                                             disable_bounds_checks=True),
        name="adaln_mqa_mixer",
    )(A_x.reshape(S // 16, 16, D), A_wq, A_wk.T, A_wv.T, A_wo, B_w1.T, B_b1,
      B_w2.reshape(FT, 16, S), B_b2, c, w_mod.reshape(D // 16, 16, 6 * D),
      grad_out.reshape(S, D))
    out, dx, dwq, dwkT, dwvT, dwo, dw1T, db1, dw2, db2, dc, dwmod = outs[:12]
    return (out.reshape(1, S, D), dx.reshape(1, S, D), dwq, dwkT.T, dwvT.T, dwo, dw1T.T,
            db1, dw2, db2, dc, dwmod.reshape(D, 6 * D))
```
